```python
import os as _os
_os.environ.setdefault("JAX_PLATFORMS", "cpu")
import jax
import jax.numpy as jnp

def _softmax(x, axis=-1):
    return jax.nn.softmax(x, axis=axis)
def _gelu(x):
    return jax.nn.gelu(x, approximate=True)
def _silu(x):
    return jax.nn.silu(x)
def _sigmoid(x):
    return jax.nn.sigmoid(x)
def _layernorm(x, axis=-1, eps=1e-5):
    m = jnp.mean(x, axis=axis, keepdims=True)
    v = jnp.var(x, axis=axis, keepdims=True)
    return (x - m) / jnp.sqrt(v + eps)
def _scatter_add(tgt, idx, src, axis=0):
    return tgt.at[idx].add(src)
def _segment_sum(src, seg, n):
    return jax.ops.segment_sum(src, seg, n)
class _Rng:
    def __init__(self, key):
        self._k = key
    def _next(self):
        self._k, sub = jax.random.split(self._k)
        return sub
    def normal(self, shape):
        return jax.random.normal(self._next(), shape, dtype=jnp.bfloat16)
    def randint(self, lo, hi, shape):
        return jax.random.randint(self._next(), shape, lo, hi, dtype=jnp.int32)
    def uniform(self, shape, lo=0.0, hi=1.0):
        return jax.random.uniform(self._next(), shape, jnp.bfloat16, lo, hi)
    def permutation(self, n):
        return jax.random.permutation(self._next(), n)


kernel_name = 'gated_mix__sliding_local_dilated__moe_arch_mod__prompt'

def setup_inputs():
    _rng = _Rng(jax.random.key(int.from_bytes(__import__("os").urandom(4), "little")))
    _w = (lambda a: (lambda t: t.astype(jnp.bfloat16) if jnp.issubdtype(t.dtype, jnp.floating) else t)(jnp.asarray(a)))
    def _A_setup():
        B, S, D = 1, 2048, 640
        return {
            "x": _w((lambda *s: _rng.normal(s) * 0.05)(B, S, D)),
            "wqkv": _w((lambda *s: _rng.normal(s) * 0.8)(D, 3 * D)),
            "wo": _w((lambda *s: _rng.normal(s) * 0.05)(D, D)),
        }
    _A_in = _A_setup()

    def _B_setup():
        B, S, D, F, C = 1, 2048, 640, 1728, 1
        return {
            "x": _w((lambda *s: _rng.normal(s) * 0.05)(B, S, D)),
            "w_r": _w((lambda *s: _rng.normal(s) * 1.6)(D)),
            "w_gate": _w((lambda *s: _rng.normal(s) * 0.4)(D, F)),
            "w_up": _w((lambda *s: _rng.normal(s) * 0.4)(D, F)),
            "w_down": _w((lambda *s: _rng.normal(s) * 0.4)(F, D)),
        }
    _B_in = _B_setup()

    return {
        "A_x": _A_in["x"],
        "A_wqkv": _A_in["wqkv"],
        "A_wo": _A_in["wo"],
        "B_x": _B_in["x"],
        "B_w_r": _B_in["w_r"],
        "B_w_gate": _B_in["w_gate"],
        "B_w_up": _B_in["w_up"],
        "B_w_down": _B_in["w_down"],
        "gate_w": _w((lambda *s: _rng.normal(s) * 0.05)(640) * 16.0),
    }

def reference(A_x, A_wqkv, A_wo, B_x, B_w_r, B_w_gate, B_w_up, B_w_down, gate_w):
    def _A_ref(x, wqkv, wo):
        B, S, D = x.shape
        H = 32; Dh = D // H
        W, dil = 8, 2
        qkv = (lambda x, *d: x.transpose(*d))((x @ wqkv).reshape(B, S, 3, H, Dh), 2, 0, 3, 1, 4)
        q, k, v = qkv[0], qkv[1], qkv[2]
        scale = Dh ** -0.5
        pos = jnp.arange(S)
        off = jnp.arange(W) * dil
        idx = pos[:, None] - off[None, :]
        mask = idx >= 0
        idx_c = jnp.where(mask, idx, 0).reshape(-1)
        kg = k[:, :, idx_c, :].reshape(B, H, S, W, Dh)
        vg = v[:, :, idx_c, :].reshape(B, H, S, W, Dh)
        logits = jnp.einsum("bhsd,bhswd->bhsw", q, kg) * scale
        logits = jnp.where(mask[None, None, :, :], logits, -1e9)
        attn = _softmax(logits, axis=-1)
        o = jnp.einsum("bhsw,bhswd->bhsd", attn, vg)
        return (lambda x, *d: x.transpose(*d))(o, 0, 2, 1, 3).reshape(B, S, D) @ wo

    def _B_ref(x, w_r, w_gate, w_up, w_down):
        B, S, D = x.shape
        C = 1
        r = x @ w_r
        idx = jnp.argsort(-r, axis=-1)[:, :C]
        idx_e = jnp.repeat(idx.reshape(B, C, 1), D, axis=2)
        x_sel = jnp.take_along_axis(x, idx_e, axis=1)
        g = _silu(x_sel @ w_gate)
        u = x_sel @ w_up
        y = (g * u) @ w_down
        r_sel = _sigmoid(jnp.take_along_axis(r, idx, axis=1))
        y = y * r_sel.reshape(B, C, 1)
        b_off = (jnp.arange(B) * S).reshape(B, 1)
        flat_idx = (idx + b_off).reshape(B * C)
        zero = (x * 0.0).reshape(B * S, D)
        upd = _scatter_add(zero, flat_idx, y.reshape(B * C, D), axis=0)
        return x + upd.reshape(B, S, D)

    x = A_x
    g = _sigmoid((x * gate_w).sum(-1, keepdims=True))
    a = _A_ref(x, A_wqkv, A_wo)
    b = _B_ref(x, B_w_r, B_w_gate, B_w_up, B_w_down)
    return g * a + (1 - g) * b
```

```python
import functools
import jax
import jax.numpy as jnp
from jax import lax
import jax.experimental.pallas as pl
import jax.experimental.pallas.tpu as pltpu

S, D, H, DH, W, DIL, F = 2048, 640, 32, 20, 8, 2, 1728
M = 256
MS = 128
NB = S // M
HALO = 16
NT = D // 128
RG = 8
FS = 16
FFN_STAGES = (3, 4, 5)
FC = F // len(FFN_STAGES)
ORDER = 'wp'
SPAN = 90
WKJ = 3
X0J = 2
A0 = 160
f32, bf16, u32, i32 = jnp.float32, jnp.bfloat16, jnp.uint32, jnp.int32
LOG2E = 1.4426950408889634
C_EXP = float(DH ** -0.5) * LOG2E
NT_DIMS = (((1,), (1,)), ((), ()))
P = functools.partial


def _kernel(x_hbm, wqkv_hbm, wo_hbm, wr_hbm, wg_hbm, wu_hbm, wd_hbm, gw_hbm, out_hbm,
            x_v, wqkv_v, wo_v, wg_v, wu_v, wd_v, tmp_v, wT_v, woP_v,
            q_v, k_v, v_v, o_v, wr_v, gw_v, zs_ref, g_v, y_v, out_v, sx, sw, sf, so):
    def cols(j):
        return pl.ds(j * 128, 128)

    def x_copies(i):
        return [pltpu.make_async_copy(x_hbm.at[0, pl.ds(i * M, M), cols(j)], x_v.at[j, pl.ds(i * M, M)], sx.at[i])
                for j in range(NT)]

    def wq_copy(j):
        return pltpu.make_async_copy(wqkv_hbm.at[cols(j), pl.ds(0, D)], wqkv_v.at[0, cols(j)], sw.at[3 + j])

    def w_copy(t):
        return pltpu.make_async_copy(wqkv_hbm.at[:, pl.ds(t * D, D)], wqkv_v.at[t], sw.at[t])

    wo_copy = pltpu.make_async_copy(wo_hbm, wo_v, sw.at[0])

    def f_copies(c):
        return [pltpu.make_async_copy(h.at[pl.ds(c * FC, FC)], v.at[pl.ds(c * FC, FC)], sf.at[c])
                for h, v in ((wg_hbm, wg_v), (wu_hbm, wu_v), (wd_hbm, wd_v))]

    def o_copies(hb):
        return [pltpu.make_async_copy(out_v.at[j, pl.ds(hb * MS, MS)], out_hbm.at[0, pl.ds(hb * MS, MS), cols(j)], so.at[hb])
                for j in range(NT)]

    def start(cs):
        for c in cs:
            c.start()

    def wait(cs):
        for c in cs:
            c.wait()

    x_u = x_v.bitcast(u32)
    out_u = out_v.bitcast(u32)
    zs_ref[0] = 0
    zs = zs_ref[0]

    def ld(ref, j, r0, n, off=0):
        return pltpu.bitcast(ref[j, pl.ds(r0 // 2 + off, n // 2), :], bf16)

    def pk(v):
        return pltpu.bitcast(v.astype(bf16), u32)

    def prep_w(t, j):
        tmp_v[j] = wqkv_v[t, j * 128:(j + 1) * 128, :].astype(f32).T
        for d in range(DH):
            wT_v[j, pl.ds((t * D + d * H) // 2, H // 2), :] = pk(tmp_v[j, pl.ds(d, H, stride=DH), :])

    def prep_wo(j):
        tmp_v[j] = wo_v[:, j * 128:(j + 1) * 128].astype(f32)
        for d in range(DH):
            woP_v[j, pl.ds(d * H // 2, H // 2), :] = pk(tmp_v[j, pl.ds(d, H, stride=DH), :])

    def proj_piece(i, t, n, m0):
        xb = jnp.concatenate([ld(x_u, j, i * M + m0, MS) for j in range(NT)], axis=1)
        wt = jnp.concatenate([ld(wT_v, j, t * D + n * 128, 128, zs if m0 else 0) for j in range(NT)], axis=1)
        (q_v, k_v, v_v)[t][n, pl.ds((HALO if t else 0) + i * M + m0, MS), :] = lax.dot_general(xb, wt, NT_DIMS, preferred_element_type=f32)

    def proj_pieces(i, ts=(0, 1, 2), row_major=False):
        if row_major:
            return [P(proj_piece, i, t, n, m0) for m0 in range(0, M, MS) for t in ts for n in range(NT)]
        return [P(proj_piece, i, t, n, m0) for t in ts for n in range(NT) for m0 in range(0, M, MS)]

    def koff(r0, w):
        o = HALO + r0 - DIL * w
        return o + zs if w >= W // 2 else o

    def probs(r0):
        q = [q_v[j, pl.ds(r0, RG), :] for j in range(NT)]
        ls = [functools.reduce(jnp.add, [q[j] * k_v[j, pl.ds(koff(r0, w), RG), :] for j in range(NT)])
              for w in range(W)]
        ls = [a + b for a, b in zip(ls, [pltpu.roll(a, 64, 1) for a in ls])]
        ls = [a + b for a, b in zip(ls, [pltpu.roll(a, 32, 1) for a in ls])]
        ls = [a * C_EXP for a in ls]
        if r0 < HALO:
            row = r0 + lax.broadcasted_iota(i32, (RG, 128), 0)
            ls = [jnp.where(row >= DIL * w, a, -1e9 * LOG2E) if r0 < DIL * w else a for w, a in enumerate(ls)]
        m = functools.reduce(jnp.maximum, ls)
        ps = [jnp.exp2(a - m) for a in ls]
        return ps, 1.0 / functools.reduce(jnp.add, ps)

    def attn_piece(r0):
        rs = range(r0, r0 + 16, RG)
        sm = [probs(r) for r in rs]
        for j in range(NT):
            os_ = [functools.reduce(jnp.add, [ps[w] * v_v[j, pl.ds(koff(r, w), RG), :] for w in range(W)]) * inv
                   for (ps, inv), r in zip(sm, rs)]
            o_v[j, pl.ds(r0 // 2, 8), :] = pk(jnp.concatenate(os_, axis=0))

    def attn_pieces(lo, hi):
        return [P(attn_piece, r0) for r0 in range(lo, hi, 16)]

    def wo_piece(i, n, m0, send):
        r0 = i * M + m0
        ob = jnp.concatenate([ld(o_v, j, r0, MS) for j in range(NT)], axis=1)
        a = jnp.dot(ob, ld(woP_v, n, 0, D, zs if m0 else 0), preferred_element_type=f32)
        xf = ld(x_u, n, r0, MS).astype(f32)
        out_u[n, pl.ds(r0 // 2, MS // 2), :] = pk(xf + g_v[pl.ds(r0, MS), :] * (a - xf))
        if send and n == NT - 1:
            start(o_copies(r0 // MS))

    def wo_pieces(i, lo=0, hi=M, send=True):
        return [P(wo_piece, i, n, m0, send) for m0 in range(lo, hi, MS) for n in range(NT)]

    def run(mm, *others, span=SPAN):
        jobs = {}
        for li, l in enumerate(others):
            for n, fn in enumerate(l):
                jobs.setdefault(int((n + 0.5 * (li > 0)) * len(mm) * span / 100 / len(l)), []).append(fn)
        for n, fn in enumerate(mm):
            fn()
            for job in jobs.get(n, ()):
                job()

    small = [pltpu.make_async_copy(wr_hbm, wr_v, sw.at[3 + NT]), pltpu.make_async_copy(gw_hbm, gw_v, sw.at[3 + NT])]
    st = dict(best=jnp.full((16, 128), -jnp.inf, f32), bidx=jnp.zeros((16, 128), i32))

    def router_piece(r0, nr):
        wr, gw = st["wr"], st["gw"]
        for rr in range(r0, r0 + nr, 16):
            xf = [ld(x_u, j, rr, 16).astype(f32) for j in range(NT)]
            rp = functools.reduce(jnp.add, [xf[j] * wr[:, j * 128:(j + 1) * 128] for j in range(NT)])
            gp = functools.reduce(jnp.add, [xf[j] * gw[:, j * 128:(j + 1) * 128] for j in range(NT)])
            r = jnp.broadcast_to(jnp.sum(rp, axis=1, keepdims=True), (16, 128))
            gl = jnp.broadcast_to(jnp.sum(gp, axis=1, keepdims=True), (16, 128))
            g_v[pl.ds(rr, 16), :] = jax.nn.sigmoid(gl)
            upd = r > st["best"]
            st["best"] = jnp.where(upd, r, st["best"])
            st["bidx"] = jnp.where(upd, rr, st["bidx"])

    def router_pieces(lo, hi, nr=32):
        return [P(router_piece, r0, nr) for r0 in range(lo * M, hi * M, nr)]

    def router_final():
        bidx = st["bidx"] + lax.broadcasted_iota(i32, (16, 128), 0)
        rmax = jnp.max(st["best"])
        idx = jnp.min(jnp.where(st["best"] == rmax, bidx, S - 1))
        base = pl.multiple_of((idx >> 4) << 4, 16)
        sel = lax.broadcasted_iota(i32, (16, 128), 0) == (idx - base)
        st.update(rmax=rmax, base=base, sel=sel, xs=jnp.concatenate([
            jnp.sum(jnp.where(sel, x_v[j, pl.ds(base, 16), :].astype(f32), 0.0), axis=0, keepdims=True)
            for j in range(NT)], axis=1))

    def ffn_piece(r0):
        rows = pl.ds(r0, FS)
        hg = jnp.sum(wg_v[rows, :].astype(f32) * st["xs"], axis=1, keepdims=True)
        hu = jnp.sum(wu_v[rows, :].astype(f32) * st["xs"], axis=1, keepdims=True)
        h = hg * jax.nn.sigmoid(hg) * hu
        t = wd_v[rows, :].astype(f32) * h
        y_v[...] += jnp.sum(t.reshape(FS // 8, 8, D), axis=0)

    def ffn_pieces(c):
        return [P(ffn_piece, r0) for r0 in range(c * FC, (c + 1) * FC, FS)]

    for j in range(NT):
        wq_copy(j).start()

    for j in range(NT):
        if j == X0J:
            start(x_copies(0))
        if j == WKJ:
            w_copy(1).start()
        wq_copy(j).wait()
        prep_w(0, j)

    start(x_copies(1))
    start(small)
    wait(x_copies(0))
    run(proj_pieces(0, (0,)))

    w_copy(2).start()
    w_copy(1).wait()
    wait(x_copies(1))
    run(proj_pieces(1, (0,)), [P(prep_w, 1, j) for j in range(NT)], span=70)

    wo_copy.start()
    for i in range(2, 4):
        start(x_copies(i))
    w_copy(2).wait()
    wait(small)
    st["wr"] = wr_v[...].astype(f32).reshape(1, D)
    st["gw"] = gw_v[...].astype(f32).reshape(1, D)
    run(proj_pieces(0, (1,)), [P(prep_w, 2, j) for j in range(NT)])
    run(proj_pieces(0, (2,)), router_pieces(0, 1))
    for j in range(NT):
        k_v[j, pl.ds(0, HALO), :] = jnp.zeros((HALO, 128), f32)
        v_v[j, pl.ds(0, HALO), :] = jnp.broadcast_to(v_v[j, pl.ds(HALO, 1), :], (HALO, 128))
    y_v[...] = jnp.zeros((8, D), f32)

    for i in range(4, NB):
        start(x_copies(i))
    wo_copy.wait()
    run(proj_pieces(1, (1, 2)), attn_pieces(0, A0), [P(prep_wo, j) for j in range(NT)])

    for i in range(1, NB - 1):
        if i + 1 in FFN_STAGES:
            start(f_copies(FFN_STAGES.index(i + 1)))
        lo = i * M
        if i == 1:
            for b in range(2, 4):
                wait(x_copies(b))
            extra = router_pieces(1, 4)
            lo = A0
        elif i == 2:
            for b in range(4, NB):
                wait(x_copies(b))
            extra = router_pieces(4, NB) + [router_final]
        elif i in FFN_STAGES:
            wait(f_copies(FFN_STAGES.index(i)))
            extra = ffn_pieces(FFN_STAGES.index(i))
        if i == 1:
            run(proj_pieces(i + 1) + wo_pieces(i - 1), attn_pieces(lo, (i + 1) * M), extra)
        elif i < NB - 2:
            pp, ww = proj_pieces(i + 1), wo_pieces(i - 1)
            run(pp + ww if ORDER == "pw" else ww + pp, attn_pieces(lo, (i + 1) * M), extra)
        else:
            for hb in range(2 * (NB - 4)):
                wait(o_copies(hb))
            run(proj_pieces(i + 1, row_major=True) + wo_pieces(i - 1),
                attn_pieces(lo, (i + 1) * M + MS), span=98)

    for hb in range(2 * (NB - 4), 2 * (NB - 3)):
        wait(o_copies(hb))
    run(wo_pieces(NB - 2) + wo_pieces(NB - 1, 0, MS), attn_pieces(S - MS, S), span=75)
    run(wo_pieces(NB - 1, MS, M, send=False))
    y = jnp.sum(y_v[...], axis=0, keepdims=True) * jax.nn.sigmoid(jnp.full((1, D), st["rmax"], f32))
    base, sel = st["base"], st["sel"]
    g = g_v[pl.ds(base, 16), :]

    for hb in range(2 * (NB - 3), 2 * NB - 1):
        wait(o_copies(hb))
    for j in range(NT):
        old = out_v[j, pl.ds(base, 16), :].astype(f32)
        out_v[j, pl.ds(base, 16), :] = jnp.where(
            sel, old + (1.0 - g) * y[:, j * 128:(j + 1) * 128], old).astype(bf16)
    start(o_copies(2 * NB - 1))

    @pl.when(base < S - MS)
    def _():
        pcs = [pltpu.make_async_copy(out_v.at[j, pl.ds(base, 16)], out_hbm.at[0, pl.ds(base, 16), cols(j)], so.at[0])
               for j in range(NT)]
        start(pcs)
        wait(pcs)
    wait(o_copies(2 * NB - 1))


@jax.jit
def pallas_gated_mix__sliding_local_dilated__moe_arch_mod__prompt_kernel(
        A_x, A_wqkv, A_wo, B_x, B_w_r, B_w_gate, B_w_up, B_w_down, gate_w):
    hbm = pl.BlockSpec(memory_space=pltpu.HBM)
    qs = pltpu.VMEM((NT, S, 128), f32)
    ks = pltpu.VMEM((NT, S + HALO, 128), f32)
    os_ = pltpu.VMEM((NT, S // 2, 128), u32)
    return pl.pallas_call(
        _kernel,
        out_shape=jax.ShapeDtypeStruct((1, S, D), bf16),
        in_specs=[hbm] * 8,
        out_specs=hbm,
        scratch_shapes=[
            pltpu.VMEM((NT, S, 128), bf16), pltpu.VMEM((3, D, D), bf16), pltpu.VMEM((D, D), bf16),
            pltpu.VMEM((F, D), bf16), pltpu.VMEM((F, D), bf16), pltpu.VMEM((F, D), bf16),
            pltpu.VMEM((NT, D, 128), f32), pltpu.VMEM((NT, 3 * D // 2, 128), u32), pltpu.VMEM((NT, D // 2, 128), u32),
            qs, ks, ks, os_, pltpu.VMEM((D,), bf16), pltpu.VMEM((D,), bf16), pltpu.SMEM((1,), i32),
            pltpu.VMEM((S, 128), f32), pltpu.VMEM((8, D), f32), pltpu.VMEM((NT, S, 128), bf16),
            pltpu.SemaphoreType.DMA((NB,)), pltpu.SemaphoreType.DMA((4 + NT,)),
            pltpu.SemaphoreType.DMA((len(FFN_STAGES),)), pltpu.SemaphoreType.DMA((2 * NB,)),
        ],
        compiler_params=pltpu.CompilerParams(vmem_limit_bytes=100 * 1024 * 1024),
    )(A_x, A_wqkv, A_wo, B_w_r, B_w_gate.T, B_w_up.T, B_w_down, gate_w)
```

```python
import functools
import jax
import jax.numpy as jnp
from jax import lax
import jax.experimental.pallas as pl
import jax.experimental.pallas.tpu as pltpu

S, D, H, DH, W, DIL, F = 2048, 640, 32, 20, 8, 2, 1728
M = 256
MS = 128
NB = S // M
HALO = 16
NT = D // 128
FS = 32
FFN_STAGES = (3, 4, 5)
FC = F // len(FFN_STAGES)
SPAN = 90
f32, bf16, u32, i32 = jnp.float32, jnp.bfloat16, jnp.uint32, jnp.int32
LOG2E = 1.4426950408889634
C_EXP = float(DH ** -0.5) * LOG2E
NT_DIMS = (((1,), (1,)), ((), ()))
P = functools.partial


def _add(xs):
    return functools.reduce(jnp.add, xs)


def _recip(s):
    r = pl.reciprocal(s, approx=True)
    return r * (2.0 - s * r)


def _sigmoid(x):
    return 0.5 * jnp.tanh(0.5 * x) + 0.5


def _kernel(x_hbm, wqkv_hbm, wo_hbm, wr_hbm, wg_hbm, wu_hbm, wd_hbm, gw_hbm, out_hbm,
            x_v, wqkv_v, wo_v, wg_v, wu_v, wd_v, tmp_v, wT_v, woP_v,
            q_v, k_v, v_v, o_v, wr_v, gw_v, g_v, y_v, out_v, sx, sw, sf, so):
    def cols(j):
        return pl.ds(j * 128, 128)

    def x_copies(i):
        return [pltpu.make_async_copy(x_hbm.at[0, pl.ds(i * M, M), cols(j)], x_v.at[j, pl.ds(i * M, M)], sx.at[i])
                for j in range(NT)]

    def wq_copy(j):
        return pltpu.make_async_copy(wqkv_hbm.at[cols(j), pl.ds(0, D)], wqkv_v.at[0, cols(j)], sw.at[3 + j])

    def w_copy(t):
        return pltpu.make_async_copy(wqkv_hbm.at[:, pl.ds(t * D, D)], wqkv_v.at[t], sw.at[t])

    wo_copy = pltpu.make_async_copy(wo_hbm, wo_v, sw.at[0])
    vec_copies = [pltpu.make_async_copy(wr_hbm, wr_v, sw.at[3 + NT]),
                  pltpu.make_async_copy(gw_hbm, gw_v, sw.at[4 + NT])]

    def f_copies(c):
        return [pltpu.make_async_copy(h.at[pl.ds(c * FC, FC)], v.at[pl.ds(c * FC, FC)], sf.at[c])
                for h, v in ((wg_hbm, wg_v), (wu_hbm, wu_v), (wd_hbm, wd_v))]

    def o_copies(hb):
        return [pltpu.make_async_copy(out_v.at[j, pl.ds(hb * 128, 128)], out_hbm.at[0, pl.ds(hb * 128, 128), cols(j)],
                                      so.at[hb]) for j in range(NT)]

    def start(cs):
        for c in cs:
            c.start()

    def wait(cs):
        for c in cs:
            c.wait()

    x_u = x_v.bitcast(u32)
    out_u = out_v.bitcast(u32)

    def ld(ref, j, r0, n):
        return pltpu.bitcast(ref[j, pl.ds(r0 // 2, n // 2), :], bf16)

    def pk(v):
        return pltpu.bitcast(v.astype(bf16), u32)

    def prep_w(t, j):
        tmp_v[j] = wqkv_v[t, j * 128:(j + 1) * 128, :].astype(f32).T
        for d in range(DH):
            wT_v[j, pl.ds((t * D + d * H) // 2, H // 2), :] = pk(tmp_v[j, pl.ds(d, H, stride=DH), :])

    def prep_wo(j):
        tmp_v[j] = wo_v[:, j * 128:(j + 1) * 128].astype(f32)
        for d in range(DH):
            woP_v[j, pl.ds(d * H // 2, H // 2), :] = pk(tmp_v[j, pl.ds(d, H, stride=DH), :])

    def proj_piece(i, t, n, m0):
        xb = jnp.concatenate([ld(x_u, j, i * M + m0, MS) for j in range(NT)], axis=1)
        wt = jnp.concatenate([ld(wT_v, j, t * D + n * 128, 128) for j in range(NT)], axis=1)
        (q_v, k_v, v_v)[t][n, pl.ds((HALO if t else 0) + i * M + m0, MS), :] = lax.dot_general(
            xb, wt, NT_DIMS, preferred_element_type=f32)

    def proj_pieces(i, ts=(0, 1, 2), row_major=False):
        if row_major:
            return [P(proj_piece, i, t, n, m0) for m0 in range(0, M, MS) for t in ts for n in range(NT)]
        return [P(proj_piece, i, t, n, m0) for t in ts for n in range(NT) for m0 in range(0, M, MS)]

    def wo_piece(n, r0, send):
        ob = jnp.concatenate([ld(o_v, j, r0, 128) for j in range(NT)], axis=1)
        a = jnp.dot(ob, ld(woP_v, n, 0, D), preferred_element_type=f32)
        xf = ld(x_u, n, r0, 128).astype(f32)
        out_u[n, pl.ds(r0 // 2, 64), :] = pk(xf + g_v[pl.ds(r0, 128), :] * (a - xf))
        if send and n == NT - 1:
            start(o_copies(r0 // 128))

    def wo_pieces(lo, hi, send=True):
        return [P(wo_piece, n, r0, send) for r0 in range(lo, hi, 128) for n in range(NT)]

    def win(ref, j, r0, w, n):
        return ref[j, pl.ds(HALO + r0 - DIL * w, n), :]

    def probs(r0, n):
        q = [q_v[j, pl.ds(r0, n), :] for j in range(NT)]
        ls = [_add([q[j] * win(k_v, j, r0, w, n) for j in range(NT)]) for w in range(W)]
        ls = [a + b for a, b in zip(ls, [pltpu.roll(a, 64, 1) for a in ls])]
        ls = [a + b for a, b in zip(ls, [pltpu.roll(a, 32, 1) for a in ls])]
        ls = [a * C_EXP for a in ls]
        if r0 < HALO:
            row = r0 + lax.broadcasted_iota(i32, (n, 128), 0)
            ls = [jnp.where(row >= DIL * w, a, -1e9 * LOG2E) if r0 < DIL * w else a for w, a in enumerate(ls)]
        m = functools.reduce(jnp.maximum, ls)
        ps = [jnp.exp2(a - m) for a in ls]
        return ps, _recip(_add(ps))

    def attn_piece(r0, n):
        rs = range(r0, r0 + 16, n)
        sm = [probs(r, n) for r in rs]
        for j in range(NT):
            os_ = [_add([ps[w] * win(v_v, j, r, w, n) for w in range(W)]) * inv for (ps, inv), r in zip(sm, rs)]
            o_v[j, pl.ds(r0 // 2, 8), :] = pk(jnp.concatenate(os_, axis=0))

    def attn_pieces(lo, hi, n=8):
        return [P(attn_piece, r0, n) for r0 in range(lo, hi, 16)]

    st = dict(best=jnp.full((16, 128), -jnp.inf, f32), bidx=jnp.zeros((16, 128), i32))

    def router_piece(r0):
        for rr in range(r0, r0 + 32, 16):
            xf = [ld(x_u, j, rr, 16).astype(f32) for j in range(NT)]
            rp = _add([xf[j] * st["wr"][:, j * 128:(j + 1) * 128] for j in range(NT)])
            gp = _add([xf[j] * st["gw"][:, j * 128:(j + 1) * 128] for j in range(NT)])
            r = jnp.broadcast_to(jnp.sum(rp, axis=1, keepdims=True), (16, 128))
            g_v[pl.ds(rr, 16), :] = _sigmoid(jnp.broadcast_to(jnp.sum(gp, axis=1, keepdims=True), (16, 128)))
            upd = r > st["best"]
            st["best"] = jnp.where(upd, r, st["best"])
            st["bidx"] = jnp.where(upd, rr, st["bidx"])

    def router_pieces(lo, hi):
        return [P(router_piece, r0) for r0 in range(lo * M, hi * M, 32)]

    def router_final():
        row = lax.broadcasted_iota(i32, (16, 128), 0)
        rmax = jnp.max(st["best"])
        idx = jnp.min(jnp.where(st["best"] == rmax, st["bidx"] + row, S - 1))
        base = pl.multiple_of((idx >> 4) << 4, 16)
        sel = row == (idx - base)
        st.update(rmax=rmax, base=base, sel=sel, xs=jnp.concatenate([
            jnp.sum(jnp.where(sel, x_v[j, pl.ds(base, 16), :].astype(f32), 0.0), axis=0, keepdims=True)
            for j in range(NT)], axis=1))

    def ffn_piece(r0):
        rows = pl.ds(r0, FS)
        hg = jnp.sum(wg_v[rows, :].astype(f32) * st["xs"], axis=1, keepdims=True)
        hu = jnp.sum(wu_v[rows, :].astype(f32) * st["xs"], axis=1, keepdims=True)
        t = wd_v[rows, :].astype(f32) * (hg * _sigmoid(hg) * hu)
        y_v[...] += jnp.sum(t.reshape(FS // 8, 8, D), axis=0)

    def ffn_pieces(c):
        return [P(ffn_piece, r0) for r0 in range(c * FC, (c + 1) * FC, FS)]

    def run(mm, *others, span=SPAN):
        jobs = {}
        for li, l in enumerate(others):
            for n, fn in enumerate(l):
                jobs.setdefault(int((n + 0.5 * (li > 0)) * len(mm) * span / 100 / len(l)), []).append(fn)
        for n, fn in enumerate(mm):
            fn()
            for job in jobs.get(n, ()):
                job()

    for j in range(NT):
        wq_copy(j).start()
    for j in range(NT):
        if j == 2:
            start(x_copies(0))
        if j == 4:
            start(x_copies(1))
        wq_copy(j).wait()
        prep_w(0, j)

    w_copy(1).start()
    start(vec_copies)
    wait(x_copies(0))
    run(proj_pieces(0, (0,)))

    w_copy(2).start()
    wait(x_copies(1))
    q1 = proj_pieces(1, (0,), row_major=True)
    run(q1[:3])

    w_copy(1).wait()
    run(q1[3:], [P(prep_w, 1, j) for j in range(NT)], span=50)

    wo_copy.start()
    for i in range(2, 4):
        start(x_copies(i))
    w_copy(2).wait()
    wait(vec_copies)
    st["wr"] = wr_v[...].astype(f32).reshape(1, D)
    st["gw"] = gw_v[...].astype(f32).reshape(1, D)
    run(proj_pieces(0, (1,)), [P(prep_w, 2, j) for j in range(NT)])
    run(proj_pieces(0, (2,)), router_pieces(0, 2))
    for j in range(NT):
        k_v[j, pl.ds(0, HALO), :] = jnp.zeros((HALO, 128), f32)
        v_v[j, pl.ds(0, HALO), :] = jnp.broadcast_to(v_v[j, pl.ds(HALO, 1), :], (HALO, 128))
    y_v[...] = jnp.zeros((8, D), f32)

    for i in range(4, NB):
        start(x_copies(i))
    wo_copy.wait()
    run(proj_pieces(1, (1, 2)), attn_pieces(0, 192))

    for i in range(2, 4):
        wait(x_copies(i))
    run(proj_pieces(2) + wo_pieces(0, M), attn_pieces(192, 2 * M, 16),
        [P(prep_wo, j) for j in range(NT)] + router_pieces(2, 4))

    for i in range(2, NB - 2):
        if i + 1 in FFN_STAGES:
            start(f_copies(FFN_STAGES.index(i + 1)))
        if i in FFN_STAGES:
            wait(f_copies(FFN_STAGES.index(i)))
            extra = ffn_pieces(FFN_STAGES.index(i))
        else:
            for b in range(4, NB):
                wait(x_copies(b))
            extra = router_pieces(4, NB) + [router_final]
        run(wo_pieces((i - 1) * M, i * M) + proj_pieces(i + 1), attn_pieces(i * M, (i + 1) * M), extra)

    for hb in range(8):
        wait(o_copies(hb))
    run(proj_pieces(NB - 1, row_major=True) + wo_pieces(S - 3 * M, S - 2 * M + 128),
        attn_pieces(S - 2 * M, S - 96), span=98)

    for hb in range(8, 10):
        wait(o_copies(hb))
    run(wo_pieces(S - 2 * M + 128, S - 128), attn_pieces(S - 96, S), span=60)
    run(wo_pieces(S - 128, S, send=False))

    y = jnp.sum(y_v[...], axis=0, keepdims=True) * _sigmoid(jnp.full((1, D), st["rmax"], f32))
    base, sel = st["base"], st["sel"]
    g = g_v[pl.ds(base, 16), :]
    for hb in range(10, 15):
        wait(o_copies(hb))
    for j in range(NT):
        old = out_v[j, pl.ds(base, 16), :].astype(f32)
        out_v[j, pl.ds(base, 16), :] = jnp.where(
            sel, old + (1.0 - g) * y[:, j * 128:(j + 1) * 128], old).astype(bf16)
    start(o_copies(15))

    @pl.when(base < S - 128)
    def _():
        pcs = [pltpu.make_async_copy(out_v.at[j, pl.ds(base, 16)], out_hbm.at[0, pl.ds(base, 16), cols(j)], so.at[0])
               for j in range(NT)]
        start(pcs)
        wait(pcs)

    wait(o_copies(15))


@jax.jit
def pallas_gated_mix__sliding_local_dilated__moe_arch_mod__prompt_kernel(
        A_x, A_wqkv, A_wo, B_x, B_w_r, B_w_gate, B_w_up, B_w_down, gate_w):
    del B_x
    hbm = pl.BlockSpec(memory_space=pltpu.HBM)
    kv = pltpu.VMEM((NT, S + HALO, 128), f32)
    return pl.pallas_call(
        _kernel,
        out_shape=jax.ShapeDtypeStruct((1, S, D), bf16),
        in_specs=[hbm] * 8,
        out_specs=hbm,
        scratch_shapes=[
            pltpu.VMEM((NT, S, 128), bf16), pltpu.VMEM((3, D, D), bf16), pltpu.VMEM((D, D), bf16),
            pltpu.VMEM((F, D), bf16), pltpu.VMEM((F, D), bf16), pltpu.VMEM((F, D), bf16),
            pltpu.VMEM((NT, D, 128), f32), pltpu.VMEM((NT, 3 * D // 2, 128), u32), pltpu.VMEM((NT, D // 2, 128), u32),
            pltpu.VMEM((NT, S, 128), f32), kv, kv, pltpu.VMEM((NT, S // 2, 128), u32),
            pltpu.VMEM((D,), bf16), pltpu.VMEM((D,), bf16),
            pltpu.VMEM((S, 128), f32), pltpu.VMEM((8, D), f32), pltpu.VMEM((NT, S, 128), bf16),
            pltpu.SemaphoreType.DMA((NB,)), pltpu.SemaphoreType.DMA((5 + NT,)),
            pltpu.SemaphoreType.DMA((len(FFN_STAGES),)), pltpu.SemaphoreType.DMA((2 * NB,)),
        ],
        compiler_params=pltpu.CompilerParams(vmem_limit_bytes=100 * 1024 * 1024),
    )(A_x, A_wqkv, A_wo, B_w_r, B_w_gate.T, B_w_up.T, B_w_down, gate_w)
```

```python
import functools
import jax
import jax.numpy as jnp
from jax import lax
import jax.experimental.pallas as pl
import jax.experimental.pallas.tpu as pltpu

S, D, H, DH, W, DIL, F = 2048, 640, 32, 20, 8, 2, 1728
M = 256
MS = 128
NB = S // M
HALO = 16
NT = D // 128
FS = 32
FFN_STAGES = (3, 4, 5)
X_GROUPS = (0, 256, 512, 1024, S)
O_GROUPS = (0, 1024, 1280, S - 128, S)
FC = F // len(FFN_STAGES)
SPAN = 90
f32, bf16, u32, i32 = jnp.float32, jnp.bfloat16, jnp.uint32, jnp.int32
LOG2E = 1.4426950408889634
C_EXP = float(DH ** -0.5) * LOG2E
NT_DIMS = (((1,), (1,)), ((), ()))
P = functools.partial


def _add(xs):
    return functools.reduce(jnp.add, xs)


def _recip(s):
    r = pl.reciprocal(s, approx=True)
    return r * (2.0 - s * r)


def _sigmoid(x):
    return 0.5 * jnp.tanh(0.5 * x) + 0.5


def _kernel(x_hbm, wqkv_hbm, wo_hbm, wr_hbm, wg_hbm, wu_hbm, wd_hbm, gw_hbm, out_hbm,
            x_v, xp_v, wqkv_v, wo_v, wg_v, wu_v, wd_v, tmp_v, wT_v, woP_v,
            q_v, k_v, v_v, o_v, wr_v, gw_v, g_v, y_v, out_v, sx, sw, sf, so):
    def cols(j):
        return pl.ds(j * 128, 128)

    def x_start(g):
        rows = pl.ds(X_GROUPS[g], X_GROUPS[g + 1] - X_GROUPS[g])
        for j in range(NT):
            pltpu.make_async_copy(x_hbm.at[0, rows, cols(j)], x_v.at[j, rows], sx.at[g]).start()

    def x_wait(g):
        dst = x_v.at[:, pl.ds(X_GROUPS[g], X_GROUPS[g + 1] - X_GROUPS[g])]
        pltpu.make_async_copy(dst, dst, sx.at[g]).wait()

    def wq_copy(j):
        return pltpu.make_async_copy(wqkv_hbm.at[cols(j), pl.ds(0, D)], wqkv_v.at[0, cols(j)], sw.at[3 + j])

    def w_copy(t):
        return pltpu.make_async_copy(wqkv_hbm.at[:, pl.ds(t * D, D)], wqkv_v.at[t], sw.at[t])

    wo_copy = pltpu.make_async_copy(wo_hbm, wo_v, sw.at[0])
    vec_copies = [pltpu.make_async_copy(wr_hbm, wr_v, sw.at[3 + NT]),
                  pltpu.make_async_copy(gw_hbm, gw_v, sw.at[4 + NT])]

    def f_copies(c):
        return [pltpu.make_async_copy(h.at[pl.ds(c * FC, FC)], v.at[pl.ds(c * FC, FC)], sf.at[c])
                for h, v in ((wg_hbm, wg_v), (wu_hbm, wu_v), (wd_hbm, wd_v))]

    def o_start(r0, n, sem):
        for j in range(NT):
            pltpu.make_async_copy(out_v.at[j, pl.ds(r0, n)], out_hbm.at[0, pl.ds(r0, n), cols(j)], sem).start()

    def o_wait(r0, n, sem):
        src = out_v.at[:, pl.ds(r0, n)]
        pltpu.make_async_copy(src, src, sem).wait()

    def o_wait_group(g):
        o_wait(O_GROUPS[g], O_GROUPS[g + 1] - O_GROUPS[g], so.at[g])

    def start(cs):
        for c in cs:
            c.start()

    def wait(cs):
        for c in cs:
            c.wait()

    def ldx(j, r0, n):
        return ld(xp_v, j, r0, n)

    def pack_x(lo, hi):
        for j in range(NT):
            xp_v[j, pl.ds(lo // 2, (hi - lo) // 2), :] = pltpu.bitcast(x_v[j, pl.ds(lo, hi - lo), :], u32)

    def ld(ref, j, r0, n):
        return pltpu.bitcast(ref[j, pl.ds(r0 // 2, n // 2), :], bf16)

    def pk(v):
        return pltpu.bitcast(v.astype(bf16), u32)

    def prep_w(t, j):
        tmp_v[j] = wqkv_v[t, j * 128:(j + 1) * 128, :].astype(f32).T
        for d in range(DH):
            wT_v[j, pl.ds((t * D + d * H) // 2, H // 2), :] = pk(tmp_v[j, pl.ds(d, H, stride=DH), :])

    def prep_wo(j):
        tmp_v[j] = wo_v[:, j * 128:(j + 1) * 128].astype(f32)
        for d in range(DH):
            woP_v[j, pl.ds(d * H // 2, H // 2), :] = pk(tmp_v[j, pl.ds(d, H, stride=DH), :])

    def proj_piece(i, t, n, m0):
        xb = jnp.concatenate([ldx(j, i * M + m0, MS) for j in range(NT)], axis=1)
        wt = jnp.concatenate([ld(wT_v, j, t * D + n * 128, 128) for j in range(NT)], axis=1)
        (q_v, k_v, v_v)[t][n, pl.ds((HALO if t else 0) + i * M + m0, MS), :] = lax.dot_general(
            xb, wt, NT_DIMS, preferred_element_type=f32)

    def proj_pieces(i, ts=(0, 1, 2), row_major=False):
        if row_major:
            return [P(proj_piece, i, t, n, m0) for m0 in range(0, M, MS) for t in ts for n in range(NT)]
        return [P(proj_piece, i, t, n, m0) for t in ts for n in range(NT) for m0 in range(0, M, MS)]

    def wo_piece(n, r0, send):
        ob = jnp.concatenate([ld(o_v, j, r0, 128) for j in range(NT)], axis=1)
        a = jnp.dot(ob, ld(woP_v, n, 0, D), preferred_element_type=f32)
        xf = x_v[n, pl.ds(r0, 128), :].astype(f32)
        out_v[n, pl.ds(r0, 128), :] = (xf + g_v[pl.ds(r0, 128), :] * (a - xf)).astype(bf16)
        if send and n == NT - 1:
            o_start(r0, 128, so.at[max(g for g, lo in enumerate(O_GROUPS) if lo <= r0)])

    def wo_pieces(lo, hi, send=True):
        return [P(wo_piece, n, r0, send) for r0 in range(lo, hi, 128) for n in range(NT)]

    def win(ref, j, r0, w, n):
        return ref[j, pl.ds(HALO + r0 - DIL * w, n), :]

    def probs(r0, n):
        q = [q_v[j, pl.ds(r0, n), :] for j in range(NT)]
        ls = [_add([q[j] * win(k_v, j, r0, w, n) for j in range(NT)]) for w in range(W)]
        ls = [a + b for a, b in zip(ls, [pltpu.roll(a, 64, 1) for a in ls])]
        ls = [a + b for a, b in zip(ls, [pltpu.roll(a, 32, 1) for a in ls])]
        ls = [a * C_EXP for a in ls]
        if r0 < HALO:
            row = r0 + lax.broadcasted_iota(i32, (n, 128), 0)
            ls = [jnp.where(row >= DIL * w, a, -1e9 * LOG2E) if r0 < DIL * w else a for w, a in enumerate(ls)]
        m = functools.reduce(jnp.maximum, ls)
        ps = [jnp.exp2(a - m) for a in ls]
        return ps, _recip(_add(ps))

    def attn_piece(r0, n):
        rs = range(r0, r0 + 16, n)
        sm = [probs(r, n) for r in rs]
        for j in range(NT):
            os_ = [_add([ps[w] * win(v_v, j, r, w, n) for w in range(W)]) * inv for (ps, inv), r in zip(sm, rs)]
            o_v[j, pl.ds(r0 // 2, 8), :] = pk(jnp.concatenate(os_, axis=0))

    def attn_pieces(lo, hi, n=8):
        return [P(attn_piece, r0, n) for r0 in range(lo, hi, 16)]

    st = dict(best=jnp.full((16, 128), -jnp.inf, f32), bidx=jnp.zeros((16, 128), i32))

    def router_piece(r0):
        for rr in range(r0, r0 + 32, 16):
            xf = [x_v[j, pl.ds(rr, 16), :].astype(f32) for j in range(NT)]
            rp = _add([xf[j] * st["wr"][:, j * 128:(j + 1) * 128] for j in range(NT)])
            gp = _add([xf[j] * st["gw"][:, j * 128:(j + 1) * 128] for j in range(NT)])
            r = jnp.broadcast_to(jnp.sum(rp, axis=1, keepdims=True), (16, 128))
            g_v[pl.ds(rr, 16), :] = _sigmoid(jnp.broadcast_to(jnp.sum(gp, axis=1, keepdims=True), (16, 128)))
            upd = r > st["best"]
            st["best"] = jnp.where(upd, r, st["best"])
            st["bidx"] = jnp.where(upd, rr, st["bidx"])

    def router_pieces(lo, hi):
        return [P(router_piece, r0) for r0 in range(lo * M, hi * M, 32)]

    def router_final():
        row = lax.broadcasted_iota(i32, (16, 128), 0)
        rmax = jnp.max(st["best"])
        idx = jnp.min(jnp.where(st["best"] == rmax, st["bidx"] + row, S - 1))
        base = pl.multiple_of((idx >> 4) << 4, 16)
        sel = row == (idx - base)
        st.update(rmax=rmax, base=base, sel=sel, xs=jnp.concatenate([
            jnp.sum(jnp.where(sel, x_v[j, pl.ds(base, 16), :].astype(f32), 0.0), axis=0, keepdims=True)
            for j in range(NT)], axis=1))

    def ffn_piece(r0):
        rows = pl.ds(r0, FS)
        hg = jnp.sum(wg_v[rows, :].astype(f32) * st["xs"], axis=1, keepdims=True)
        hu = jnp.sum(wu_v[rows, :].astype(f32) * st["xs"], axis=1, keepdims=True)
        t = wd_v[rows, :].astype(f32) * (hg * _sigmoid(hg) * hu)
        y_v[...] += jnp.sum(t.reshape(FS // 8, 8, D), axis=0)

    def ffn_pieces(c):
        return [P(ffn_piece, r0) for r0 in range(c * FC, (c + 1) * FC, FS)]

    def run(mm, *others, span=SPAN):
        jobs = {}
        for li, l in enumerate(others):
            for n, fn in enumerate(l):
                jobs.setdefault(int((n + 0.5 * (li > 0)) * len(mm) * span / 100 / len(l)), []).append(fn)
        for n, fn in enumerate(mm):
            fn()
            for job in jobs.get(n, ()):
                job()

    for j in range(NT):
        wq_copy(j).start()
    for j in range(NT):
        if j == 2:
            x_start(0)
        if j == 4:
            x_start(1)
        wq_copy(j).wait()
        prep_w(0, j)

    w_copy(1).start()
    start(vec_copies)
    x_wait(0)
    pack_x(0, M)
    run(proj_pieces(0, (0,)))

    w_copy(2).start()
    x_wait(1)
    pack_x(M, 2 * M)
    q1 = proj_pieces(1, (0,), row_major=True)
    run(q1[:3])

    w_copy(1).wait()
    run(q1[3:], [P(prep_w, 1, j) for j in range(NT)], span=50)

    wo_copy.start()
    x_start(2)
    w_copy(2).wait()
    wait(vec_copies)
    st["wr"] = wr_v[...].astype(f32).reshape(1, D)
    st["gw"] = gw_v[...].astype(f32).reshape(1, D)
    run(proj_pieces(0, (1,)), [P(prep_w, 2, j) for j in range(NT)])
    run(proj_pieces(0, (2,)), router_pieces(0, 2))
    for j in range(NT):
        k_v[j, pl.ds(0, HALO), :] = jnp.zeros((HALO, 128), f32)
        v_v[j, pl.ds(0, HALO), :] = jnp.broadcast_to(v_v[j, pl.ds(HALO, 1), :], (HALO, 128))
    y_v[...] = jnp.zeros((8, D), f32)

    x_start(3)
    wo_copy.wait()
    run(proj_pieces(1, (1, 2)), attn_pieces(0, 192, 16))

    x_wait(2)
    pack_x(2 * M, 3 * M)
    run(proj_pieces(2) + wo_pieces(0, M), attn_pieces(192, 2 * M, 16),
        [P(prep_wo, j) for j in range(NT)] + router_pieces(2, 4), span=98)

    for i in range(2, NB - 2):
        if i + 1 in FFN_STAGES:
            start(f_copies(FFN_STAGES.index(i + 1)))
        if i in FFN_STAGES:
            wait(f_copies(FFN_STAGES.index(i)))
            extra = ffn_pieces(FFN_STAGES.index(i))
        else:
            x_wait(3)
            extra = router_pieces(4, NB) + [router_final]
        pack_x((i + 1) * M, (i + 2) * M)
        run(wo_pieces((i - 1) * M, i * M) + proj_pieces(i + 1), attn_pieces(i * M, (i + 1) * M), extra,
            span=SPAN if i in FFN_STAGES else 80)

    o_wait_group(0)
    pack_x(S - M, S)
    run(proj_pieces(NB - 1), attn_pieces(S - 2 * M, S - M, 16))

    o_wait_group(1)
    run(wo_pieces(S - 3 * M, S - 128), attn_pieces(S - M, S), span=85)
    run(wo_pieces(S - 128, S, send=False))

    y = jnp.sum(y_v[...], axis=0, keepdims=True) * _sigmoid(jnp.full((1, D), st["rmax"], f32))
    base, sel = st["base"], st["sel"]
    g = g_v[pl.ds(base, 16), :]
    o_wait_group(2)
    for j in range(NT):
        old = out_v[j, pl.ds(base, 16), :].astype(f32)
        out_v[j, pl.ds(base, 16), :] = jnp.where(
            sel, old + (1.0 - g) * y[:, j * 128:(j + 1) * 128], old).astype(bf16)
    o_start(S - 128, 128, so.at[3])

    @pl.when(base < S - 128)
    def _():
        o_start(base, 16, so.at[0])
        o_wait(base, 16, so.at[0])

    o_wait_group(3)


@jax.jit
def pallas_gated_mix__sliding_local_dilated__moe_arch_mod__prompt_kernel(
        A_x, A_wqkv, A_wo, B_x, B_w_r, B_w_gate, B_w_up, B_w_down, gate_w):
    del B_x
    hbm = pl.BlockSpec(memory_space=pltpu.HBM)
    kv = pltpu.VMEM((NT, S + HALO, 128), f32)
    return pl.pallas_call(
        _kernel,
        out_shape=jax.ShapeDtypeStruct((1, S, D), bf16),
        in_specs=[hbm] * 8,
        out_specs=hbm,
        scratch_shapes=[
            pltpu.VMEM((NT, S, 128), bf16), pltpu.VMEM((NT, S // 2, 128), u32),
            pltpu.VMEM((3, D, D), bf16), pltpu.VMEM((D, D), bf16),
            pltpu.VMEM((F, D), bf16), pltpu.VMEM((F, D), bf16), pltpu.VMEM((F, D), bf16),
            pltpu.VMEM((NT, D, 128), f32), pltpu.VMEM((NT, 3 * D // 2, 128), u32), pltpu.VMEM((NT, D // 2, 128), u32),
            pltpu.VMEM((NT, S, 128), f32), kv, kv, pltpu.VMEM((NT, S // 2, 128), u32),
            pltpu.VMEM((D,), bf16), pltpu.VMEM((D,), bf16),
            pltpu.VMEM((S, 128), f32), pltpu.VMEM((8, D), f32), pltpu.VMEM((NT, S, 128), bf16),
            pltpu.SemaphoreType.DMA((4,)), pltpu.SemaphoreType.DMA((5 + NT,)),
            pltpu.SemaphoreType.DMA((len(FFN_STAGES),)), pltpu.SemaphoreType.DMA((4,)),
        ],
        compiler_params=pltpu.CompilerParams(
            vmem_limit_bytes=100 * 1024 * 1024,
            flags={"XLA_TPU_EVENLY_DISTRIBUTE_CRITICAL_NODES": True}),
    )(A_x, A_wqkv, A_wo, B_w_r, B_w_gate.T, B_w_up.T, B_w_down, gate_w)
```
